```python
import jax
import jax.numpy as jnp

def _softmax(x, axis=-1):
    return jax.nn.softmax(x, axis=axis)

def _gelu(x):
    return jax.nn.gelu(x, approximate=True)

def _silu(x):
    return jax.nn.silu(x)

def _sigmoid(x):
    return jax.nn.sigmoid(x)

def _layernorm(x, axis=-1, eps=1e-05):
    m = jnp.mean(x, axis=axis, keepdims=True)
    v = jnp.var(x, axis=axis, keepdims=True)
    return (x - m) / jnp.sqrt(v + eps)

def _scatter_add(tgt, idx, src, axis=0):
    return tgt.at[idx].add(src)

def _segment_sum(src, seg, n):
    return jax.ops.segment_sum(src, seg, n)

class _Rng:

    def __init__(self, key):
        self._k = key

    def _next(self):
        self._k, sub = jax.random.split(self._k)
        return sub

    def normal(self, shape):
        return jax.random.normal(self._next(), shape, dtype=jnp.bfloat16)

    def randint(self, lo, hi, shape):
        return jax.random.randint(self._next(), shape, lo, hi, dtype=jnp.int32)

    def uniform(self, shape, lo=0.0, hi=1.0):
        return jax.random.uniform(self._next(), shape, jnp.bfloat16, lo, hi)

    def permutation(self, n):
        return jax.random.permutation(self._next(), n)
kernel_name = 'adaLN_cond__sliding_block_cached__mixer_token_mlp__decode'

def setup_inputs():
    _rng = _Rng(jax.random.key(int.from_bytes(__import__("os").urandom(4), "little")))
    _w = lambda a: (lambda t: t.astype(jnp.bfloat16) if jnp.issubdtype(t.dtype, jnp.floating) else t)(jnp.asarray(a))

    def _A_setup():
        B, Sq, D = (1, 1, 640)
        Hq, Hkv, Sk, Dh = (32, 32, 32768, 192)
        assert Hq % Hkv == 0, (Hq, Hkv)
        return {'x': _w((lambda *s: _rng.normal(s) * 0.05)(B, Sq, D)), 'k_cache': _w((lambda *s: _rng.normal(s) * 0.05)(B, Hkv, Sk, Dh)), 'v_cache': _w((lambda *s: _rng.normal(s) * 0.05)(B, Hkv, Sk, Dh)), 'wq': _w((lambda *s: _rng.normal(s) * 0.05)(D, Hq * Dh) * D ** (-0.5)), 'wo': _w((lambda *s: _rng.normal(s) * 0.05)(Hq * Dh, D) * (Hq * Dh) ** (-0.5))}
    _A_in = _A_setup()

    def _B_setup():
        B, S, D, F = (1, 1, 640, 1536)
        return {'x': _w((lambda *s: _rng.normal(s) * 0.05)(B, S, D)), 'w1': _w((lambda *s: _rng.normal(s) * 0.05)(S, F) * S ** (-0.5)), 'b1': _w((lambda *s: _rng.normal(s) * 0.05)(F) * 0.02), 'w2': _w((lambda *s: _rng.normal(s) * 0.05)(F, S) * F ** (-0.5)), 'b2': _w((lambda *s: _rng.normal(s) * 0.05)(S) * 0.02)}
    _B_in = _B_setup()
    return {'A_x': _A_in['x'], 'A_k_cache': _A_in['k_cache'], 'A_v_cache': _A_in['v_cache'], 'A_wq': _A_in['wq'], 'A_wo': _A_in['wo'], 'B_x': _B_in['x'], 'B_w1': _B_in['w1'], 'B_b1': _B_in['b1'], 'B_w2': _B_in['w2'], 'B_b2': _B_in['b2'], 'c': _w((lambda *s: _rng.normal(s) * 0.05)(1, 640)), 'w_mod': _w((lambda *s: _rng.normal(s) * 0.05)(640, 6 * 640) * 640 ** (-0.5))}

def reference(A_x, A_k_cache, A_v_cache, A_wq, A_wo, B_x, B_w1, B_b1, B_w2, B_b2, c, w_mod):

    def _A_ref(x, k_cache, v_cache, wq, wo):
        B, Sq, D = x.shape
        Hq, Dh = (32, 192)
        Hkv, Sk = (k_cache.shape[1], k_cache.shape[2])
        W = min(4096, max(256, Sk // 4))
        rep = Hq // Hkv
        q = (lambda x, *d: x.transpose(*d))((x @ wq).reshape(B, Sq, Hq, Dh), 0, 2, 1, 3)
        k = jnp.repeat(k_cache[:, :, Sk - W:, :], rep, axis=1)
        v = jnp.repeat(v_cache[:, :, Sk - W:, :], rep, axis=1)
        scores = jnp.einsum('bhqd,bhkd->bhqk', q, k) * Dh ** (-0.5)
        p = _softmax(scores, axis=-1)
        o = jnp.einsum('bhqk,bhkd->bhqd', p, v)
        return (lambda x, *d: x.transpose(*d))(o, 0, 2, 1, 3).reshape(B, Sq, Hq * Dh) @ wo

    def _B_ref(x, w1, b1, w2, b2):
        B, S, D = x.shape
        h = _layernorm(x, axis=-1)
        u = jnp.einsum('bsd,sf->bdf', h, w1) + b1
        u = _gelu(u)
        y = jnp.einsum('bdf,fs->bds', u, w2) + b2
        return (lambda x, *d: x.transpose(*d))(y, 0, 2, 1)
    x = A_x
    mod = (_silu(c) @ w_mod).reshape(c.shape[0], 6, 1, -1)
    sa, ca, ga, sb, cb, gb = (mod[:, 0].copy(), mod[:, 1].copy(), mod[:, 2].copy(), mod[:, 3].copy(), mod[:, 4].copy(), mod[:, 5].copy())
    h = _layernorm(x, axis=-1) * (1 + ca) + sa
    x = x + ga * _A_ref(h, A_k_cache, A_v_cache, A_wq, A_wo)
    h = _layernorm(x, axis=-1) * (1 + cb) + sb
    x = x + gb * _B_ref(h, B_w1, B_b1, B_w2, B_b2)
    return x
```

```python
import jax
import jax.numpy as jnp
import jax.experimental.pallas as pl
import jax.experimental.pallas.tpu as pltpu

D = 640
H = 32
DH = 192
SK = 32768
W = min(4096, max(256, SK // 4))
F = 1536
NS = 3
EPS = 1e-5
F32 = jnp.float32
BF16 = jnp.bfloat16


def _ln(x):
    m = jnp.mean(x, axis=-1, keepdims=True)
    xc = x - m
    v = jnp.mean(xc * xc, axis=-1, keepdims=True)
    return xc / jnp.sqrt(v + EPS)


def _col_bcast(row):
    return jnp.broadcast_to(row, (128, 128)).T


def _kernel(x_hbm, kt_hbm, vt_hbm, wq_hbm, wo_hbm, w1_hbm, b1_hbm, w2_hbm, b2_hbm,
            c_hbm, wm_hbm, o_ref,
            x_v, c_v, w1_v, b1_v, w2_v, b2_v, wm_v, wq_v, wo_v, kbuf, vbuf,
            qb, w1b, b1b, w2b, sem_s, sem_w, sem_k, sem_v):
    def k_copy(h, slot):
        return pltpu.make_async_copy(
            kt_hbm.at[0, h, :, pl.ds(SK - W, W)], kbuf.at[slot], sem_k.at[slot])

    def v_copy(h, slot):
        return pltpu.make_async_copy(
            vt_hbm.at[0, h, :, pl.ds(SK - W, W)], vbuf.at[slot], sem_v.at[slot])

    def wm_copy(lo, hi, i):
        return pltpu.make_async_copy(
            wm_hbm.at[:, pl.ds(lo, hi - lo)], wm_v.at[:, pl.ds(lo, hi - lo)], sem_w.at[i])

    small = [pltpu.make_async_copy(s, d, sem_s.at[i]) for i, (s, d) in enumerate(
        [(c_hbm, c_v), (x_hbm, x_v), (w1_hbm, w1_v), (b1_hbm, b1_v), (w2_hbm, w2_v),
         (b2_hbm, b2_v)])]
    wm_a = wm_copy(0, 2 * D, 0)
    wm_b = wm_copy(2 * D, 5 * D, 1)
    wm_c = wm_copy(5 * D, 6 * D, 2)
    wq_c = pltpu.make_async_copy(wq_hbm, wq_v, sem_w.at[3])
    wo_c = pltpu.make_async_copy(wo_hbm, wo_v, sem_w.at[4])

    for s in small:
        s.start()
    wm_a.start()
    wq_c.start()
    k_copy(0, 0).start()
    wo_c.start()
    v_copy(0, 0).start()
    for i in range(1, NS):
        k_copy(i, i).start()
        v_copy(i, i).start()
    wm_b.start()
    for s in small:
        s.wait()

    w1r = w1_v[...].astype(F32)
    w2r = w2_v[...].astype(F32) * 0.5
    b1r = b1_v[...].astype(F32).reshape(1, F)
    for j in range(F // 128):
        sl = slice(j * 128, (j + 1) * 128)
        w1b[sl, :] = _col_bcast(w1r[:, sl])
        w2b[sl, :] = _col_bcast(w2r[:, sl])
        b1b[sl, :] = _col_bcast(b1r[:, sl])
    lin1 = jnp.sum(w1r * w2r, axis=-1, keepdims=True)
    lin0 = jnp.sum(b1r * w2r, axis=-1, keepdims=True) + b2_v[...].astype(F32).reshape(1, 1)

    cf = c_v[...].astype(F32)
    sc = (cf * jax.nn.sigmoid(cf)).astype(BF16)
    x0 = x_v[0].astype(F32)
    wm_a.wait()
    mod_a = jnp.dot(sc, wm_v[:, 0:2 * D], preferred_element_type=F32)
    h1 = _ln(x0) * (1.0 + mod_a[:, D:2 * D]) + mod_a[:, 0:D]
    wq_c.wait()
    q = jnp.dot(h1.astype(BF16), wq_v[...], preferred_element_type=F32) * (DH ** -0.5)
    for j in range(H * DH // 128):
        sl = slice(j * 128, (j + 1) * 128)
        qb[sl, :] = _col_bcast(q[:, sl])
    wo_c.wait()

    NC = W // 128

    def head(h, yacc):
        slot = h % NS
        row0 = pl.multiple_of(h * DH, DH)
        k_copy(h, slot).wait()
        qh = qb[pl.ds(row0, DH), :]
        s = []
        for j in range(NC):
            kt = kbuf[slot, :, j * 128:(j + 1) * 128].astype(F32)
            s.append(jnp.sum(kt * qh, axis=0, keepdims=True))

        @pl.when(h + NS < H)
        def _():
            k_copy(h + NS, slot).start()

        m = s[0]
        for j in range(1, NC):
            m = jnp.maximum(m, s[j])
        m = jnp.max(m, axis=-1, keepdims=True)
        p = [jnp.exp(sj - m) for sj in s]
        l = p[0]
        for j in range(1, NC):
            l = l + p[j]
        l = jnp.sum(l, axis=-1, keepdims=True)

        v_copy(h, slot).wait()
        acc = vbuf[slot, :, 0:128].astype(F32) * p[0]
        for j in range(1, NC):
            acc = acc + vbuf[slot, :, j * 128:(j + 1) * 128].astype(F32) * p[j]

        @pl.when(h + NS < H)
        def _():
            v_copy(h + NS, slot).start()

        @pl.when(h + NS == H - 1)
        def _():
            wm_c.start()

        o = jnp.sum(acc, axis=-1, keepdims=True) / l
        contrib = wo_v[pl.ds(row0, DH), :].astype(F32) * o
        return yacc + jnp.sum(contrib.reshape(DH // 8, 8, D), axis=0)

    yacc = lax_fori(H, head, jnp.zeros((8, D), F32))
    attn = jnp.sum(yacc, axis=0, keepdims=True)

    wm_b.wait()
    mod_b = jnp.dot(sc, wm_v[:, 2 * D:5 * D], preferred_element_type=F32)
    x1 = x0 + mod_b[:, 0:D] * attn
    h2 = _ln(x1) * (1.0 + mod_b[:, 2 * D:3 * D]) + mod_b[:, D:2 * D]
    hn = _ln(h2)
    hb = jnp.broadcast_to(hn, (8, D))

    c0 = 0.7978845608028654
    c1 = c0 * 0.044715

    def mlp(g, acc):
        r = pl.multiple_of(g * 8, 8)
        w1g = jnp.tile(w1b[pl.ds(r, 8), :], (1, D // 128))
        b1g = jnp.tile(b1b[pl.ds(r, 8), :], (1, D // 128))
        w2g = jnp.tile(w2b[pl.ds(r, 8), :], (1, D // 128))
        u = hb * w1g + b1g
        t = jnp.tanh(u * (c0 + c1 * (u * u)))
        return acc + (u * w2g) * t

    macc = jax.lax.fori_loop(0, F // 8, mlp, jnp.zeros((8, D), F32), unroll=8)
    y = jnp.sum(macc, axis=0, keepdims=True) + hn * lin1 + lin0

    wm_c.wait()
    gb = jnp.dot(sc, wm_v[:, 5 * D:6 * D], preferred_element_type=F32)
    o_ref[0] = (x1 + gb * y).astype(o_ref.dtype)


def lax_fori(n, body, init):
    return jax.lax.fori_loop(0, n, body, init)


@jax.jit
def pallas_adaLN_cond__sliding_block_cached__mixer_token_mlp__decode_kernel(
    A_x, A_k_cache, A_v_cache, A_wq, A_wo, B_x, B_w1, B_b1, B_w2, B_b2, c, w_mod,
):
    del B_x
    kt = jnp.swapaxes(A_k_cache, 2, 3)
    vt = jnp.swapaxes(A_v_cache, 2, 3)
    w2 = B_w2.reshape(1, F)
    any_spec = pl.BlockSpec(memory_space=pl.ANY)
    return pl.pallas_call(
        _kernel,
        out_shape=jax.ShapeDtypeStruct((1, 1, D), A_x.dtype),
        in_specs=[any_spec] * 11,
        out_specs=pl.BlockSpec(memory_space=pltpu.VMEM),
        scratch_shapes=[
            pltpu.VMEM((1, 1, D), BF16), pltpu.VMEM((1, D), BF16),
            pltpu.VMEM((1, F), BF16), pltpu.VMEM((F,), BF16), pltpu.VMEM((1, F), BF16),
            pltpu.VMEM((1,), BF16),
            pltpu.VMEM((D, 6 * D), BF16), pltpu.VMEM((D, H * DH), BF16),
            pltpu.VMEM((H * DH, D), BF16),
            pltpu.VMEM((NS, DH, W), BF16), pltpu.VMEM((NS, DH, W), BF16),
            pltpu.VMEM((H * DH, 128), F32),
            pltpu.VMEM((F, 128), F32), pltpu.VMEM((F, 128), F32), pltpu.VMEM((F, 128), F32),
            pltpu.SemaphoreType.DMA((6,)), pltpu.SemaphoreType.DMA((5,)),
            pltpu.SemaphoreType.DMA((NS,)), pltpu.SemaphoreType.DMA((NS,)),
        ],
        compiler_params=pltpu.CompilerParams(vmem_limit_bytes=64 * 2**20),
    )(A_x, kt, vt, A_wq, A_wo, B_w1, B_b1, w2, B_b2, c, w_mod)
```

```python
import jax
import jax.numpy as jnp
import jax.experimental.pallas as pl
import jax.experimental.pallas.tpu as pltpu

D = 640
H = 32
DH = 192
SK = 32768
W = min(4096, max(256, SK // 4))
F = 1536
NS = 2
EPS = 1e-5
C0 = 0.7978845608028654
KS = (C0 * 0.044715) ** (1.0 / 3.0)
F32 = jnp.float32
BF16 = jnp.bfloat16


def _ln(x):
    m = jnp.mean(x, axis=-1, keepdims=True)
    xc = x - m
    v = jnp.mean(xc * xc, axis=-1, keepdims=True)
    return xc / jnp.sqrt(v + EPS)


def _col_bcast(row):
    return jnp.broadcast_to(row, (128, 128)).T


def _kernel(x_hbm, kt_hbm, vt_hbm, wq_hbm, wo_hbm, w1_hbm, b1_hbm, w2_hbm, b2_hbm,
            c_hbm, wm_hbm, o_ref,
            x_v, c_v, w1_v, b1_v, w2_v, b2_v, wm_v, wq_v, wo_v, kbuf, vbuf,
            qb, w1b, b1b, w2b, sem_s, sem_w, sem_k, sem_v):
    def k_copy(h, slot):
        return pltpu.make_async_copy(
            kt_hbm.at[0, h, :, pl.ds(SK - W, W)], kbuf.at[slot], sem_k.at[slot])

    def v_copy(h, slot):
        return pltpu.make_async_copy(
            vt_hbm.at[0, h, :, pl.ds(SK - W, W)], vbuf.at[slot], sem_v.at[slot])

    def wm_copy(lo, hi, i):
        return pltpu.make_async_copy(
            wm_hbm.at[:, pl.ds(lo, hi - lo)], wm_v.at[:, pl.ds(lo, hi - lo)], sem_w.at[i])

    small = [pltpu.make_async_copy(s, d, sem_s.at[i]) for i, (s, d) in enumerate(
        [(c_hbm, c_v), (x_hbm, x_v), (w1_hbm, w1_v), (b1_hbm, b1_v), (w2_hbm, w2_v),
         (b2_hbm, b2_v)])]
    wm_a = wm_copy(0, 2 * D, 0)
    wm_b = wm_copy(2 * D, 5 * D, 1)
    wm_c = wm_copy(5 * D, 6 * D, 2)
    wq_c = pltpu.make_async_copy(wq_hbm, wq_v, sem_w.at[3])
    wo_c = pltpu.make_async_copy(wo_hbm, wo_v, sem_w.at[4])

    for s in small:
        s.start()
    wm_a.start()
    wq_c.start(priority=1)
    k_copy(0, 0).start()
    wo_c.start(priority=1)
    v_copy(0, 0).start(priority=1)
    for i in range(1, NS):
        k_copy(i, i).start()
        v_copy(i, i).start(priority=1)
    wm_b.start()
    for s in small:
        s.wait()

    w1r = w1_v[...].astype(F32) * KS
    w2r = w2_v[...].astype(F32) * (0.5 / KS)
    b1r = b1_v[...].astype(F32).reshape(1, F) * KS
    for j in range(F // 128):
        sl = slice(j * 128, (j + 1) * 128)
        w1b[sl, :] = _col_bcast(w1r[:, sl])
        w2b[sl, :] = _col_bcast(w2r[:, sl])
        b1b[sl, :] = _col_bcast(b1r[:, sl])
    lin1 = jnp.sum(w1r * w2r, axis=-1, keepdims=True)
    lin0 = jnp.sum(b1r * w2r, axis=-1, keepdims=True) + b2_v[...].astype(F32).reshape(1, 1)

    cf = c_v[...].astype(F32)
    sc = (cf * jax.nn.sigmoid(cf)).astype(BF16)
    x0 = x_v[0].astype(F32)
    wm_a.wait()
    mod_a = jnp.dot(sc, wm_v[:, 0:2 * D], preferred_element_type=F32)
    h1 = _ln(x0) * (1.0 + mod_a[:, D:2 * D]) + mod_a[:, 0:D]
    wq_c.wait()
    q = jnp.dot(h1.astype(BF16), wq_v[...], preferred_element_type=F32) * (DH ** -0.5)
    for j in range(H * DH // 128):
        sl = slice(j * 128, (j + 1) * 128)
        qb[sl, :] = _col_bcast(q[:, sl])
    wo_c.wait()

    NC = W // 128

    def head(h, yacc):
        slot = h % NS
        row0 = pl.multiple_of(h * DH, DH)
        k_copy(h, slot).wait()
        qh = qb[pl.ds(row0, DH), :]
        s = []
        for j in range(NC):
            kt = kbuf[slot, :, j * 128:(j + 1) * 128].astype(F32)
            s.append(jnp.sum(kt * qh, axis=0, keepdims=True))

        @pl.when(h + NS < H)
        def _():
            k_copy(h + NS, slot).start()

        m = s[0]
        for j in range(1, NC):
            m = jnp.maximum(m, s[j])
        m = jnp.max(m, axis=-1, keepdims=True)
        p = [jnp.exp(sj - m) for sj in s]
        l = p[0]
        for j in range(1, NC):
            l = l + p[j]
        l = jnp.sum(l, axis=-1, keepdims=True)

        v_copy(h, slot).wait()

        @pl.when(h == H - 1)
        def _():
            wm_c.start()

        acc = vbuf[slot, :, 0:128].astype(F32) * p[0]
        for j in range(1, NC):
            acc = acc + vbuf[slot, :, j * 128:(j + 1) * 128].astype(F32) * p[j]

        @pl.when(h + NS < H)
        def _():
            v_copy(h + NS, slot).start(priority=1)

        o = jnp.sum(acc, axis=-1, keepdims=True) / l
        contrib = wo_v[pl.ds(row0, DH), :].astype(F32) * o
        return yacc + jnp.sum(contrib.reshape(DH // 8, 8, D), axis=0)

    yacc = jax.lax.fori_loop(0, H, head, jnp.zeros((8, D), F32))
    attn = jnp.sum(yacc, axis=0, keepdims=True)

    wm_b.wait()
    mod_b = jnp.dot(sc, wm_v[:, 2 * D:5 * D], preferred_element_type=F32)
    x1 = x0 + mod_b[:, 0:D] * attn
    h2 = _ln(x1) * (1.0 + mod_b[:, 2 * D:3 * D]) + mod_b[:, D:2 * D]
    hn = _ln(h2)
    hb = jnp.broadcast_to(hn, (8, D))


    def mlp(g, acc):
        r = pl.multiple_of(g * 8, 8)
        w1g = jnp.tile(w1b[pl.ds(r, 8), :], (1, D // 128))
        b1g = jnp.tile(b1b[pl.ds(r, 8), :], (1, D // 128))
        w2g = jnp.tile(w2b[pl.ds(r, 8), :], (1, D // 128))
        u = hb * w1g + b1g
        t = jnp.tanh(u * (C0 / KS + u * u))
        return acc + (u * w2g) * t

    macc = jax.lax.fori_loop(0, F // 8, mlp, jnp.zeros((8, D), F32), unroll=8)
    y = jnp.sum(macc, axis=0, keepdims=True) + hn * lin1 + lin0

    wm_c.wait()
    gb = jnp.dot(sc, wm_v[:, 5 * D:6 * D], preferred_element_type=F32)
    o_ref[0] = (x1 + gb * y).astype(o_ref.dtype)


@jax.jit
def pallas_adaLN_cond__sliding_block_cached__mixer_token_mlp__decode_kernel(
    A_x, A_k_cache, A_v_cache, A_wq, A_wo, B_x, B_w1, B_b1, B_w2, B_b2, c, w_mod,
):
    del B_x
    kt = jnp.swapaxes(A_k_cache, 2, 3)
    vt = jnp.swapaxes(A_v_cache, 2, 3)
    w2 = B_w2.reshape(1, F)
    any_spec = pl.BlockSpec(memory_space=pl.ANY)
    return pl.pallas_call(
        _kernel,
        out_shape=jax.ShapeDtypeStruct((1, 1, D), A_x.dtype),
        in_specs=[any_spec] * 11,
        out_specs=pl.BlockSpec(memory_space=pltpu.VMEM),
        scratch_shapes=[
            pltpu.VMEM((1, 1, D), BF16), pltpu.VMEM((1, D), BF16),
            pltpu.VMEM((1, F), BF16), pltpu.VMEM((F,), BF16), pltpu.VMEM((1, F), BF16),
            pltpu.VMEM((1,), BF16),
            pltpu.VMEM((D, 6 * D), BF16), pltpu.VMEM((D, H * DH), BF16),
            pltpu.VMEM((H * DH, D), BF16),
            pltpu.VMEM((NS, DH, W), BF16), pltpu.VMEM((NS, DH, W), BF16),
            pltpu.VMEM((H * DH, 128), F32),
            pltpu.VMEM((F, 128), F32), pltpu.VMEM((F, 128), F32), pltpu.VMEM((F, 128), F32),
            pltpu.SemaphoreType.DMA((6,)), pltpu.SemaphoreType.DMA((5,)),
            pltpu.SemaphoreType.DMA((NS,)), pltpu.SemaphoreType.DMA((NS,)),
        ],
        compiler_params=pltpu.CompilerParams(vmem_limit_bytes=64 * 2**20),
    )(A_x, kt, vt, A_wq, A_wo, B_w1, B_b1, w2, B_b2, c, w_mod)
```

```python
import jax
import jax.numpy as jnp
import jax.experimental.pallas as pl
import jax.experimental.pallas.tpu as pltpu

D = 640
H = 32
DH = 192
SK = 32768
W = min(4096, max(256, SK // 4))
F = 1536
NS = 2
VP = 3
VR = DH // VP
EPS = 1e-5
C0 = 0.7978845608028654
KS = (C0 * 0.044715) ** (1.0 / 3.0)
F32 = jnp.float32
BF16 = jnp.bfloat16


def _ln(x):
    m = jnp.mean(x, axis=-1, keepdims=True)
    xc = x - m
    v = jnp.mean(xc * xc, axis=-1, keepdims=True)
    return xc / jnp.sqrt(v + EPS)


def _col_bcast(row):
    return jnp.broadcast_to(row, (128, 128)).T


def _kernel(x_hbm, kt_hbm, vt_hbm, wq_hbm, wo_hbm, w1_hbm, b1_hbm, w2_hbm, b2_hbm,
            c_hbm, wm_hbm, o_ref,
            x_v, c_v, w1_v, b1_v, w2_v, b2_v, wm_v, wq_v, wo_v, kbuf, vbuf,
            qb, w1b, b1b, w2b, modb, scb, sem_s, sem_w, sem_k, sem_v):
    def k_copy(h, slot):
        return pltpu.make_async_copy(
            kt_hbm.at[0, h, :, pl.ds(SK - W, W)], kbuf.at[slot], sem_k.at[slot])

    def v_copy(h, slot, r):
        return pltpu.make_async_copy(
            vt_hbm.at[0, h, pl.ds(r * VR, VR), pl.ds(SK - W, W)],
            vbuf.at[slot, pl.ds(r * VR, VR)], sem_v.at[slot * VP + r])

    def v_start(h, slot):
        for r in range(VP):
            v_copy(h, slot, r).start(priority=1)

    def wm_copy(lo, hi, i):
        return pltpu.make_async_copy(
            wm_hbm.at[:, pl.ds(lo, hi - lo)], wm_v.at[:, pl.ds(lo, hi - lo)], sem_w.at[i])

    small = [pltpu.make_async_copy(s, d, sem_s.at[i]) for i, (s, d) in enumerate(
        [(c_hbm, c_v), (x_hbm, x_v), (w1_hbm, w1_v), (b1_hbm, b1_v), (w2_hbm, w2_v),
         (b2_hbm, b2_v)])]
    wm_a = wm_copy(0, 2 * D, 0)
    wm_b = wm_copy(2 * D, 5 * D, 1)
    wm_c = wm_copy(5 * D, 6 * D, 2)
    wq_c = pltpu.make_async_copy(wq_hbm, wq_v, sem_w.at[3])
    wo_c = pltpu.make_async_copy(wo_hbm, wo_v, sem_w.at[4])

    for s in small:
        s.start()
    wm_a.start()
    wq_c.start(priority=1)
    k_copy(0, 0).start()
    wo_c.start(priority=1)
    v_start(0, 0)
    for i in range(1, NS):
        k_copy(i, i).start()
        v_start(i, i)
    wm_b.start()
    for s in small:
        s.wait()

    w1r = w1_v[...].astype(F32) * KS
    w2r = w2_v[...].astype(F32) * (0.5 / KS)
    b1r = b1_v[...].astype(F32).reshape(1, F) * KS
    for j in range(F // 128):
        sl = slice(j * 128, (j + 1) * 128)
        w1b[sl, :] = _col_bcast(w1r[:, sl])
        w2b[sl, :] = _col_bcast(w2r[:, sl])
        b1b[sl, :] = _col_bcast(b1r[:, sl])
    lin1 = jnp.sum(w1r * w2r, axis=-1, keepdims=True)
    lin0 = jnp.sum(b1r * w2r, axis=-1, keepdims=True) + b2_v[...].astype(F32).reshape(1, 1)

    cf = c_v[...].astype(F32)
    sc = (cf * jax.nn.sigmoid(cf)).astype(BF16)
    scf = sc.astype(F32)
    for j in range(D // 128):
        sl = slice(j * 128, (j + 1) * 128)
        scb[sl, :] = _col_bcast(scf[:, sl])
    x0 = x_v[0].astype(F32)
    wm_a.wait()
    mod_a = jnp.dot(sc, wm_v[:, 0:2 * D], preferred_element_type=F32)
    h1 = _ln(x0) * (1.0 + mod_a[:, D:2 * D]) + mod_a[:, 0:D]
    wq_c.wait()
    q = jnp.dot(h1.astype(BF16), wq_v[...], preferred_element_type=F32) * (DH ** -0.5)
    for j in range(H * DH // 128):
        sl = slice(j * 128, (j + 1) * 128)
        qb[sl, :] = _col_bcast(q[:, sl])
    wo_c.wait()

    NC = W // 128

    def head(h, yacc):
        slot = h % NS
        row0 = pl.multiple_of(h * DH, DH)
        k_copy(h, slot).wait()
        qh = qb[pl.ds(row0, DH), :]
        s = []
        for j in range(NC):
            kt = kbuf[slot, :, j * 128:(j + 1) * 128].astype(F32)
            s.append(jnp.sum(kt * qh, axis=0, keepdims=True))

        @pl.when(h + NS < H)
        def _():
            k_copy(h + NS, slot).start()

        @pl.when(h == 2)
        def _():
            wm_b.wait()
            modb[...] = jnp.dot(sc, wm_v[:, 2 * D:5 * D], preferred_element_type=F32)

        m = s[0]
        for j in range(1, NC):
            m = jnp.maximum(m, s[j])
        m = jnp.max(m, axis=-1, keepdims=True)
        p = [jnp.exp(sj - m) for sj in s]
        l = p[0]
        for j in range(1, NC):
            l = l + p[j]
        l = jnp.sum(l, axis=-1, keepdims=True)

        for r in range(VP):
            v_copy(h, slot, r).wait()
            if r == VP - 1:
                @pl.when(h == H - 1)
                def _():
                    wm_c.start()
            rs = slice(r * VR, (r + 1) * VR)
            acc = vbuf[slot, rs, 0:128].astype(F32) * p[0]
            for j in range(1, NC):
                acc = acc + vbuf[slot, rs, j * 128:(j + 1) * 128].astype(F32) * p[j]
            o = jnp.sum(acc, axis=-1, keepdims=True) / l
            contrib = wo_v[pl.ds(row0 + r * VR, VR), :].astype(F32) * o
            yacc = yacc + jnp.sum(contrib.reshape(VR // 8, 8, D), axis=0)

        @pl.when(h + NS < H)
        def _():
            v_start(h + NS, slot)

        return yacc

    yacc = jax.lax.fori_loop(0, H, head, jnp.zeros((8, D), F32))
    attn = jnp.sum(yacc, axis=0, keepdims=True)

    mod_b = modb[...]
    x1 = x0 + mod_b[:, 0:D] * attn
    h2 = _ln(x1) * (1.0 + mod_b[:, 2 * D:3 * D]) + mod_b[:, D:2 * D]
    hn = _ln(h2)
    hb = jnp.broadcast_to(hn, (8, D))


    def mlp(g, acc):
        r = pl.multiple_of(g * 8, 8)
        w1g = jnp.tile(w1b[pl.ds(r, 8), :], (1, D // 128))
        b1g = jnp.tile(b1b[pl.ds(r, 8), :], (1, D // 128))
        w2g = jnp.tile(w2b[pl.ds(r, 8), :], (1, D // 128))
        u = hb * w1g + b1g
        t = jnp.tanh(u * (C0 / KS + u * u))
        return acc + (u * w2g) * t

    macc = jax.lax.fori_loop(0, F // 8, mlp, jnp.zeros((8, D), F32), unroll=8)
    y = jnp.sum(macc, axis=0, keepdims=True) + hn * lin1 + lin0

    wm_c.wait()
    sct = scb[...]
    gb = jnp.concatenate(
        [jnp.sum(wm_v[:, 5 * D + j * 128:5 * D + (j + 1) * 128].astype(F32) * sct,
                 axis=0, keepdims=True) for j in range(D // 128)], axis=-1)
    o_ref[0] = (x1 + gb * y).astype(o_ref.dtype)


@jax.jit
def pallas_adaLN_cond__sliding_block_cached__mixer_token_mlp__decode_kernel(
    A_x, A_k_cache, A_v_cache, A_wq, A_wo, B_x, B_w1, B_b1, B_w2, B_b2, c, w_mod,
):
    del B_x
    kt = jnp.swapaxes(A_k_cache, 2, 3)
    vt = jnp.swapaxes(A_v_cache, 2, 3)
    w2 = B_w2.reshape(1, F)
    any_spec = pl.BlockSpec(memory_space=pl.ANY)
    return pl.pallas_call(
        _kernel,
        out_shape=jax.ShapeDtypeStruct((1, 1, D), A_x.dtype),
        in_specs=[any_spec] * 11,
        out_specs=pl.BlockSpec(memory_space=pltpu.VMEM),
        scratch_shapes=[
            pltpu.VMEM((1, 1, D), BF16), pltpu.VMEM((1, D), BF16),
            pltpu.VMEM((1, F), BF16), pltpu.VMEM((F,), BF16), pltpu.VMEM((1, F), BF16),
            pltpu.VMEM((1,), BF16),
            pltpu.VMEM((D, 6 * D), BF16), pltpu.VMEM((D, H * DH), BF16),
            pltpu.VMEM((H * DH, D), BF16),
            pltpu.VMEM((NS, DH, W), BF16), pltpu.VMEM((NS, DH, W), BF16),
            pltpu.VMEM((H * DH, 128), F32),
            pltpu.VMEM((F, 128), F32), pltpu.VMEM((F, 128), F32), pltpu.VMEM((F, 128), F32),
            pltpu.VMEM((1, 3 * D), F32), pltpu.VMEM((D, 128), F32),
            pltpu.SemaphoreType.DMA((6,)), pltpu.SemaphoreType.DMA((5,)),
            pltpu.SemaphoreType.DMA((NS,)), pltpu.SemaphoreType.DMA((NS * VP,)),
        ],
        compiler_params=pltpu.CompilerParams(vmem_limit_bytes=64 * 2**20),
    )(A_x, kt, vt, A_wq, A_wo, B_w1, B_b1, w2, B_b2, c, w_mod)
```
